```python
import os as _os
_os.environ.setdefault('JAX_PLATFORMS', 'cpu')
import jax
import jax.numpy as jnp

def _softmax(x, axis=-1):
    return jax.nn.softmax(x, axis=axis)

def _gelu(x):
    return jax.nn.gelu(x, approximate=True)

def _silu(x):
    return jax.nn.silu(x)

def _sigmoid(x):
    return jax.nn.sigmoid(x)

def _layernorm(x, axis=-1, eps=1e-05):
    m = jnp.mean(x, axis=axis, keepdims=True)
    v = jnp.var(x, axis=axis, keepdims=True)
    return (x - m) / jnp.sqrt(v + eps)

def _scatter_add(tgt, idx, src, axis=0):
    return tgt.at[idx].add(src)

def _segment_sum(src, seg, n):
    return jax.ops.segment_sum(src, seg, n)

class _Rng:

    def __init__(self, key):
        self._k = key

    def _next(self):
        self._k, sub = jax.random.split(self._k)
        return sub

    def normal(self, shape):
        return jax.random.normal(self._next(), shape, dtype=jnp.bfloat16)

    def randint(self, lo, hi, shape):
        return jax.random.randint(self._next(), shape, lo, hi, dtype=jnp.int32)

    def uniform(self, shape, lo=0.0, hi=1.0):
        return jax.random.uniform(self._next(), shape, jnp.bfloat16, lo, hi)

    def permutation(self, n):
        return jax.random.permutation(self._next(), n)
kernel_name = 'sequential_preLN__memory_aug_recurrent_mem_tr__swiglu_ffn__prompt'

def setup_inputs():
    _rng = _Rng(jax.random.key(int.from_bytes(__import__("os").urandom(4), "little")))
    _w = lambda a: (lambda t: t.astype(jnp.bfloat16) if jnp.issubdtype(t.dtype, jnp.floating) else t)(jnp.asarray(a))

    def _A_setup():
        B, S, Dm = (1, 2048, 640)
        H, Dh = (32, 192)
        M, seg = (8, 32)
        seg = min(seg, S)
        S = S // seg * seg
        return {'x': _w((lambda *s: _rng.normal(s) * 0.05)(B, S, Dm)), 'mem0': _w((lambda *s: _rng.normal(s) * 0.1)(B, M, Dm)), 'Wq': _w((lambda *s: _rng.normal(s) * 1.6)(Dm, H, Dh) * Dm ** (-0.5)), 'Wk': _w((lambda *s: _rng.normal(s) * 1.6)(Dm, H, Dh) * Dm ** (-0.5)), 'Wv': _w((lambda *s: _rng.normal(s) * 0.1)(Dm, H, Dh) * Dm ** (-0.5)), 'Wo': _w((lambda *s: _rng.normal(s) * 0.1)(H, Dh, Dm) * (H * Dh) ** (-0.5)), 'seg_len': seg}
    _A_in = _A_setup()

    def _B_setup():
        B, S, D, F = (1, 2048, 640, 1536)
        return {'x': _w((lambda *s: _rng.normal(s) * 0.05)(B, S, D)), 'w_gate': _w((lambda *s: _rng.normal(s) * 0.05)(D, F)), 'w_up': _w((lambda *s: _rng.normal(s) * 0.05)(D, F)), 'w_down': _w((lambda *s: _rng.normal(s) * 0.05)(F, D))}
    _B_in = _B_setup()
    return {'A_x': _A_in['x'], 'A_mem0': _A_in['mem0'], 'A_Wq': _A_in['Wq'], 'A_Wk': _A_in['Wk'], 'A_Wv': _A_in['Wv'], 'A_Wo': _A_in['Wo'], 'A_seg_len': _A_in['seg_len'], 'B_x': _B_in['x'], 'B_w_gate': _B_in['w_gate'], 'B_w_up': _B_in['w_up'], 'B_w_down': _B_in['w_down']}

def reference(A_x, A_mem0, A_Wq, A_Wk, A_Wv, A_Wo, A_seg_len, B_x, B_w_gate, B_w_up, B_w_down):

    def _A_ref(x, mem0, Wq, Wk, Wv, Wo, seg_len):
        B, S, Dm = x.shape
        H, Dh = (Wq.shape[1], Wq.shape[2])
        M = mem0.shape[1]
        scale = Dh ** (-0.5)
        n_seg = S // seg_len
        L = M + seg_len
        idx = jnp.arange(L)
        mask = (idx[:, None] < M) | (idx[:, None] >= idx[None, :])
        mem = mem0
        outs = []
        for s in range(n_seg):
            xs = x[:, s * seg_len:(s + 1) * seg_len, :].copy()
            h = jnp.concatenate([mem, xs], axis=1)
            q = jnp.einsum('btd,dhe->bhte', h, Wq)
            k = jnp.einsum('btd,dhe->bhte', h, Wk)
            v = jnp.einsum('btd,dhe->bhte', h, Wv)
            scores = jnp.einsum('bhqe,bhke->bhqk', q, k) * scale
            scores = jnp.where(mask[None, None], scores, -1000000000.0)
            p = _softmax(scores, axis=-1)
            o = jnp.einsum('bhqk,bhke->bhqe', p, v)
            o = jnp.einsum('bhte,hed->btd', o, Wo)
            mem = o[:, :M, :].copy()
            outs.append(o[:, M:, :])
        return jnp.concatenate(outs, axis=1)

    def _B_ref(x, w_gate, w_up, w_down):
        g = _silu(x @ w_gate)
        u = x @ w_up
        return g * u @ w_down
    x = A_x
    h = x + _A_ref(_layernorm(x, axis=-1), A_mem0, A_Wq, A_Wk, A_Wv, A_Wo, A_seg_len)
    h2 = h + _B_ref(_layernorm(h, axis=-1), B_w_gate, B_w_up, B_w_down)
    return h2
```

```python
import functools

import jax
import jax.numpy as jnp
from jax import lax
import jax.experimental.pallas as pl
import jax.experimental.pallas.tpu as pltpu

F32 = jnp.float32
BF16 = jnp.bfloat16
U32 = jnp.uint32

LN_EPS = 1e-5
MASK_VALUE = -1000000000.0
STAGE_DEPTH = 4


def _mm(a, b):
    return lax.dot_general(a, b, (((1,), (0,)), ((), ())), preferred_element_type=F32)


def _layernorm(x):
    n = x.shape[-1]
    mean = jnp.sum(x, axis=-1, keepdims=True) * (1.0 / n)
    d = x - mean
    var = jnp.sum(d * d, axis=-1, keepdims=True) * (1.0 / n)
    return d * lax.rsqrt(var + LN_EPS)


def _kernel(x_hbm, mem0_ref, wq_hbm, wk_hbm, wv_hbm, wo_hbm, wg_hbm, wu_hbm, wd_hbm,
            out_hbm,
            stage, wqkv, wo_raw, wo_s, wg_s, wu_s, wd_s, x_s, hbuf, hres, hn, out_s,
            sem_stage, sem_misc, sem_out,
            *, n_seg, seg, n_mem, n_pair, dh, d, f_half):
    L = n_mem + seg
    pw = 2 * dh
    n_tile = pw // 128
    blk = 2 * seg
    scale = dh ** (-0.5)

    def stage_copies(g, slot):
        rows = pl.ds(pl.multiple_of(g * pw, 128), pw)
        return [pltpu.make_async_copy(w.at[rows, :], stage.at[slot, j], sem_stage.at[slot * 3 + j])
                for j, w in enumerate((wq_hbm, wk_hbm, wv_hbm))]

    x_cp = pltpu.make_async_copy(x_hbm, x_s, sem_misc.at[0])
    wo_cp = pltpu.make_async_copy(wo_hbm, wo_raw, sem_misc.at[1])
    ffn_cps = []
    for c in range(2):
        cols = pl.ds(c * f_half, f_half)
        ffn_cps.append(pltpu.make_async_copy(wg_hbm.at[:, cols], wg_s.at[c], sem_misc.at[2 + c]))
        ffn_cps.append(pltpu.make_async_copy(wu_hbm.at[:, cols], wu_s.at[c], sem_misc.at[4 + c]))
        ffn_cps.append(pltpu.make_async_copy(wd_hbm.at[cols, :], wd_s.at[c], sem_misc.at[6 + c]))

    for g in range(STAGE_DEPTH):
        for cp in stage_copies(g, g):
            cp.start()
    x_cp.start()

    hres[...] = jnp.zeros(hres.shape, hres.dtype)
    hn[...] = jnp.zeros(hn.shape, hn.dtype)

    def relayout(g, carry):
        slot = g % STAGE_DEPTH
        for cp in stage_copies(g, slot):
            cp.wait()
        for j in range(3):
            for t in range(n_tile):
                w_t = stage[slot, j, t * 128:(t + 1) * 128, :].T
                c0 = j * pw + t * 128
                wqkv[g, :, c0:c0 + 128] = pltpu.bitcast(w_t, U32)

        @pl.when(g + STAGE_DEPTH < n_pair)
        def _():
            for cp in stage_copies(g + STAGE_DEPTH, slot):
                cp.start()

        @pl.when(g + STAGE_DEPTH == n_pair)
        def _():
            wo_cp.start()

        @pl.when(g == n_pair - 1)
        def _():
            for cp in ffn_cps:
                cp.start()
        return carry

    lax.fori_loop(0, n_pair, relayout, 0)

    x_cp.wait()
    hbuf[0:n_mem, :] = mem0_ref[...].astype(F32)
    hbuf[n_mem:L, :] = _layernorm(x_s[0:seg, :].astype(F32))

    wo_cp.wait()

    def relayout_wo(g, carry):
        rows = pl.ds(pl.multiple_of(g * pw, 128), pw)
        wo_s[g] = pltpu.bitcast(wo_raw[rows, :], U32)
        return carry

    lax.fori_loop(0, n_pair, relayout_wo, 0)
    for cp in ffn_cps:
        cp.wait()

    def ffn_chunk(slot, c):
        a = hn[slot]
        gate = _mm(a, wg_s[c])
        up = _mm(a, wu_s[c])
        act = (gate * jax.nn.sigmoid(gate) * up).astype(BF16)
        return hres[slot] + _mm(act, wd_s[c])

    def out_copy(b):
        rows = pl.ds(pl.multiple_of(b * blk, blk), blk)
        return pltpu.make_async_copy(out_s.at[rows, :], out_hbm.at[rows, :], sem_out)

    def step(s, carry):
        row = lax.broadcasted_iota(jnp.int32, (L, 2 * L), 0)
        col = lax.broadcasted_iota(jnp.int32, (L, 2 * L), 1)
        first = col < L
        key = jnp.where(first, col, col - L)
        visible = (row < n_mem) | (row >= key)
        lane = lax.broadcasted_iota(jnp.int32, (L, 128), 1)
        lo = lane < (dh - 128)
        zeros = jnp.zeros((L, 128), F32)

        def block_diag(t):
            t0, t1, t2 = t[:, 0:128], t[:, 128:256], t[:, 256:384]
            top = jnp.concatenate([t0, jnp.where(lo, t1, 0.0), zeros], axis=1)
            bot = jnp.concatenate([zeros, jnp.where(lo, 0.0, t1), t2], axis=1)
            return jnp.concatenate([top, bot], axis=0).astype(BF16)

        def qkv(g):
            r = _mm(hbuf[...], pltpu.bitcast(wqkv[g], BF16))
            return r[:, 0:pw], block_diag(r[:, pw:2 * pw]), block_diag(r[:, 2 * pw:3 * pw])

        def scores(q, kb):
            sc = lax.dot_general(q, kb, (((1,), (1,)), ((), ())), preferred_element_type=F32)
            sc = jnp.where(visible, sc * scale, MASK_VALUE)
            m_a = jnp.max(jnp.where(first, sc, -jnp.inf), axis=1, keepdims=True)
            m_b = jnp.max(jnp.where(first, -jnp.inf, sc), axis=1, keepdims=True)
            e = jnp.exp(sc - jnp.where(first, m_a, m_b))
            l_a = jnp.sum(jnp.where(first, e, 0.0), axis=1, keepdims=True)
            l_b = jnp.sum(jnp.where(first, 0.0, e), axis=1, keepdims=True)
            return e / jnp.where(first, l_a, l_b)

        held, probs, outs = {}, {}, {}
        acc = None
        for i in range(n_pair + 2):
            if i < n_pair:
                held[i] = qkv(i)
            if 0 <= i - 1 < n_pair:
                probs[i - 1] = scores(held[i - 1][0], held[i - 1][1])
            if i == n_pair:
                for g in range(n_pair - 2):
                    t = _mm(outs.pop(g), pltpu.bitcast(wo_s[g], BF16))
                    acc = t if acc is None else acc + t
            if 0 <= i - 2 < n_pair:
                outs[i - 2] = _mm(probs.pop(i - 2), held.pop(i - 2)[2])
        for g in range(n_pair - 2, n_pair):
            acc = acc + _mm(outs.pop(g), pltpu.bitcast(wo_s[g], BF16))

        c = s % 2
        b = s // 2
        res = ffn_chunk((b + 1) % 2, c)
        hres[(b + 1) % 2] = res
        prev = jnp.maximum(b - 1, 0)
        out_s[pl.ds(pl.multiple_of(prev * blk, blk), blk), :] = res.astype(BF16)

        rows = pl.ds(pl.multiple_of(s * seg, seg), seg)
        h = x_s[rows, :].astype(F32) + acc[n_mem:L, :]
        half = pl.ds(pl.multiple_of(c * seg, seg), seg)
        hres[b % 2, half, :] = h
        hn[b % 2, half, :] = _layernorm(h).astype(BF16)
        nxt = jnp.minimum(s + 1, n_seg - 1)
        hbuf[0:n_mem, :] = acc[0:n_mem, :]
        hbuf[n_mem:L, :] = _layernorm(x_s[pl.ds(pl.multiple_of(nxt * seg, seg), seg), :].astype(F32))

        @pl.when((c == 1) & (b >= 1))
        def _():
            out_copy(prev).start()
        return carry

    lax.fori_loop(0, n_seg, step, 0)

    last = n_seg // 2 - 1
    hres[last % 2] = ffn_chunk(last % 2, 0)
    out_s[last * blk:(last + 1) * blk, :] = ffn_chunk(last % 2, 1).astype(BF16)
    out_copy(last).start()
    for b in range(n_seg // 2):
        out_copy(b).wait()


@functools.partial(jax.jit, static_argnames=("A_seg_len",))
def pallas_sequential_preLN__memory_aug_recurrent_mem_tr__swiglu_ffn__prompt_kernel(
    A_x: jax.Array,
    A_mem0: jax.Array,
    A_Wq: jax.Array,
    A_Wk: jax.Array,
    A_Wv: jax.Array,
    A_Wo: jax.Array,
    A_seg_len: int,
    B_x: jax.Array,
    B_w_gate: jax.Array,
    B_w_up: jax.Array,
    B_w_down: jax.Array,
):
    del B_x
    batch, seq, d = A_x.shape
    _, heads, dh = A_Wq.shape
    n_mem = A_mem0.shape[1]
    seg = int(A_seg_len)
    n_seg = seq // seg
    f = B_w_gate.shape[1]
    n_pair = heads // 2
    pw = 2 * dh
    f_half = f // 2
    assert batch == 1 and n_seg * seg == seq and n_seg % 2 == 0
    assert dh == 192 and heads % 2 == 0 and 2 * (n_mem + seg) <= 128

    wt = lambda w: jnp.transpose(w, (1, 2, 0)).reshape(heads * dh, d)

    hbm = pl.BlockSpec(memory_space=pl.ANY)
    vmem = pl.BlockSpec(memory_space=pltpu.VMEM)
    body = functools.partial(_kernel, n_seg=n_seg, seg=seg, n_mem=n_mem, n_pair=n_pair,
                             dh=dh, d=d, f_half=f_half)
    out = pl.pallas_call(
        body,
        out_shape=jax.ShapeDtypeStruct((seq, d), A_x.dtype),
        in_specs=[hbm, vmem] + [hbm] * 7,
        out_specs=hbm,
        scratch_shapes=[
            pltpu.VMEM((STAGE_DEPTH, 3, pw, d), BF16),
            pltpu.VMEM((n_pair, d // 2, 3 * pw), U32),
            pltpu.VMEM((heads * dh, d), BF16),
            pltpu.VMEM((n_pair, pw // 2, d), U32),
            pltpu.VMEM((2, d, f_half), BF16),
            pltpu.VMEM((2, d, f_half), BF16),
            pltpu.VMEM((2, f_half, d), BF16),
            pltpu.VMEM((seq, d), BF16),
            pltpu.VMEM((n_mem + seg, d), F32),
            pltpu.VMEM((2, 2 * seg, d), F32),
            pltpu.VMEM((2, 2 * seg, d), BF16),
            pltpu.VMEM((seq, d), BF16),
            pltpu.SemaphoreType.DMA((STAGE_DEPTH * 3,)),
            pltpu.SemaphoreType.DMA((8,)),
            pltpu.SemaphoreType.DMA(()),
        ],
        compiler_params=pltpu.CompilerParams(vmem_limit_bytes=100 * 1024 * 1024),
    )(A_x.reshape(seq, d), A_mem0.reshape(n_mem, d), wt(A_Wq), wt(A_Wk), wt(A_Wv),
      A_Wo.reshape(heads * dh, d), B_w_gate, B_w_up, B_w_down)
    return out.reshape(batch, seq, d)
```

```python
import functools

import jax
import jax.numpy as jnp
from jax import lax
import jax.experimental.pallas as pl
import jax.experimental.pallas.tpu as pltpu

F32 = jnp.float32
BF16 = jnp.bfloat16
U32 = jnp.uint32

LN_EPS = 1e-5
MASK_VALUE = -1000000000.0
STAGE_DEPTH = 4
PRE_ROWS = 8
UNROLL = (1, 1)
N_PRE = 43
FFN_COLS = 256
LAG_QK = 1
LAG_PV = 3


def _mm(a, b):
    return lax.dot_general(a, b, (((1,), (0,)), ((), ())), preferred_element_type=F32)


def _mm_t(a, b):
    return lax.dot_general(a, b, (((1,), (1,)), ((), ())), preferred_element_type=F32)


def _w(packed):
    return pltpu.bitcast(packed, BF16)


def _swiglu(gate, up):
    hg = 0.5 * gate
    return ((hg * jnp.tanh(hg) + hg) * up).astype(BF16)


def _recip(x):
    r = pl.reciprocal(x, approx=True)
    return r * (2.0 - x * r)


def _layernorm(x):
    n = x.shape[-1]
    mean = jnp.sum(x, axis=-1, keepdims=True) * (1.0 / n)
    d = x - mean
    var = jnp.sum(d * d, axis=-1, keepdims=True) * (1.0 / n)
    return d * lax.rsqrt(var + LN_EPS)


def _kernel(x_hbm, mem0_hbm, wq_hbm, wk_hbm, wv_hbm, wo_hbm, wg_hbm, wu_hbm, wd_hbm,
            out_hbm,
            stage, wqkv_even, wqkv_odd, wo_raw, wo_s, wg_s, wu_s, wd_s,
            x_s, x_pre, mem_s, h_pre, pre, hbuf, hres, hn, out_s,
            sem_stage, sem_wo, sem_misc, sem_out,
            *, n_seg, seg, n_mem, n_pair, dh, f_half):
    L = n_mem + seg
    pw = 2 * dh
    n_tile = pw // 128
    blk = 2 * seg
    n_blk = n_seg // 2
    scale = dh ** (-0.5)
    live = seg - PRE_ROWS

    def pair_rows(g):
        return pl.ds(pl.multiple_of(g * pw, 128), pw)

    def stage_copies(g):
        slot = g % STAGE_DEPTH
        return [pltpu.make_async_copy(w.at[pair_rows(g), :], stage.at[slot, j],
                                      sem_stage.at[slot * 3 + j])
                for j, w in enumerate((wq_hbm, wk_hbm, wv_hbm))]

    def wo_copy(g):
        return pltpu.make_async_copy(wo_hbm.at[pair_rows(g), :], wo_raw.at[g], sem_wo)

    def out_copy(b):
        rows = pl.ds(pl.multiple_of(b * blk, blk), blk)
        return pltpu.make_async_copy(out_s.at[rows, :], out_hbm.at[rows, :], sem_out)

    mem_cp = pltpu.make_async_copy(mem0_hbm, mem_s, sem_misc.at[8])
    x_head = pltpu.make_async_copy(x_hbm.at[pl.ds(0, 3)], x_s.at[pl.ds(0, 3)], sem_misc.at[0])
    x_rest = pltpu.make_async_copy(x_hbm.at[pl.ds(3, n_seg - 3)], x_s.at[pl.ds(3, n_seg - 3)],
                                   sem_misc.at[1])
    x_tail = pltpu.make_async_copy(x_hbm.at[pl.ds(1, N_PRE), pl.ds(live, PRE_ROWS), :], x_pre,
                                   sem_misc.at[9])
    ffn_cps = []
    for c in range(2):
        cols = pl.ds(c * f_half, f_half)
        ffn_cps.append(pltpu.make_async_copy(wg_hbm.at[:, cols], wg_s.at[c], sem_misc.at[2 + c]))
        ffn_cps.append(pltpu.make_async_copy(wu_hbm.at[:, cols], wu_s.at[c], sem_misc.at[4 + c]))
        ffn_cps.append(pltpu.make_async_copy(wd_hbm.at[cols, :], wd_s.at[c], sem_misc.at[6 + c]))

    def w_qkv(g):
        return _w((wqkv_odd if g % 2 else wqkv_even)[g // 2])

    def make_attention():
        row = lax.broadcasted_iota(jnp.int32, (L, 128), 0)
        col = lax.broadcasted_iota(jnp.int32, (L, 128), 1)
        first = col < L
        second = (col >= L) & (col < 2 * L)
        key = jnp.where(first, col, col - L)
        visible = (row < n_mem) | (row >= key)
        lo = col < (dh - 128)
        zeros = jnp.zeros((L, 128), F32)

        def split(r):
            k0, k1, k2, v0, v1, v2 = (r[:, t * 128:(t + 1) * 128] for t in range(n_tile, 3 * n_tile))
            k01 = jnp.concatenate([
                jnp.concatenate([k0, jnp.where(lo, k1, 0.0)], axis=1),
                jnp.concatenate([zeros, jnp.where(lo, 0.0, k1)], axis=1),
                jnp.zeros((128 - 2 * L, 256), F32)], axis=0).astype(BF16)
            k2 = jnp.concatenate([k2, jnp.zeros((128 - L, 128), F32)], axis=0).astype(BF16)
            vb = jnp.concatenate([
                jnp.concatenate([v0, jnp.where(lo, v1, 0.0), zeros], axis=1),
                jnp.concatenate([zeros, jnp.where(lo, 0.0, v1), v2], axis=1)], axis=0).astype(BF16)
            return r[:, 0:pw], (k01, k2), vb

        def probs(q, k):
            sc = _mm_t(q[:, 0:256], k[0]) + pltpu.roll(_mm_t(q[:, 256:384], k[1]), L, axis=1)
            sc = jnp.where(visible, sc * scale, MASK_VALUE)
            m_a = jnp.max(jnp.where(first, sc, -jnp.inf), axis=1, keepdims=True)
            m_b = jnp.max(jnp.where(second, sc, -jnp.inf), axis=1, keepdims=True)
            e = jnp.exp(sc - jnp.where(first, m_a, m_b))
            l_a = jnp.sum(jnp.where(first, e, 0.0), axis=1, keepdims=True)
            l_b = jnp.sum(jnp.where(second, e, 0.0), axis=1, keepdims=True)
            return (e * _recip(jnp.where(first, l_a, l_b)))[:, 0:2 * L]

        return split, probs

    def finish(s, acc, slot, c, nxt):
        hbuf[0:n_mem, :] = acc[0:n_mem, :]
        hbuf[n_mem:L, :] = _layernorm(x_s[nxt].astype(F32))
        h = x_s[s].astype(F32) + acc[n_mem:L, :]
        hres[slot, c * seg:(c + 1) * seg, :] = h
        hn[slot, c * seg:(c + 1) * seg, :] = _layernorm(h).astype(BF16)

    def step(s, slot, c, nxt, with_ffn, short):
        split, probs = make_attention()
        if short:
            h = hbuf[0:n_mem + live, :]
            ready = pl.ds(pl.multiple_of(L + (s - 1) * PRE_ROWS, PRE_ROWS), PRE_ROWS)
            project = lambda g: jnp.concatenate([_mm(h, w_qkv(g)), pre[g, ready, :]], axis=0)
        else:
            h = hbuf[...]
            project = lambda g: _mm(h, w_qkv(g))
        held, p, outs = {}, {}, {}
        for i in range(n_pair):
            held[i] = split(project(i))
            if i >= LAG_PV:
                outs[i - LAG_PV] = _mm(p.pop(i - LAG_PV), held.pop(i - LAG_PV)[2])
            if i >= LAG_QK:
                p[i - LAG_QK] = probs(held[i - LAG_QK][0], held[i - LAG_QK][1])
        acc = None
        acts = []
        if with_ffn:
            a = hn[1 - slot]
        for g in range(n_pair):
            if with_ffn and g % 3 == 0 and g // 3 < f_half // FFN_COLS:
                cs = slice((g // 3) * FFN_COLS, (g // 3 + 1) * FFN_COLS)
                acts.append(_swiglu(_mm(a, wg_s[c, :, cs]), _mm(a, wu_s[c, :, cs])))
            if g % 3 == (0 if with_ffn else 2):
                i = n_pair + g // 3
                if i - LAG_PV < n_pair:
                    outs[i - LAG_PV] = _mm(p.pop(i - LAG_PV), held.pop(i - LAG_PV)[2])
                if i - LAG_QK < n_pair:
                    p[i - LAG_QK] = probs(held[i - LAG_QK][0], held[i - LAG_QK][1])
            t = _mm(outs.pop(g), _w(wo_s[g]))
            acc = t if acc is None else acc + t
        finish(s, acc, slot, c, nxt)
        if with_ffn:
            return hres[1 - slot] + _mm(jnp.concatenate(acts, axis=1), wd_s[c])

    for cp in [mem_cp, x_head, x_tail] + stage_copies(0):
        cp.start()
    mem_cp.wait()
    x_head.wait()
    for cp in stage_copies(1):
        cp.start()
    x_tail.wait()
    tail = lambda i: x_pre[i - 1].astype(F32)
    first_rows = jnp.concatenate([mem_s[...].astype(F32), _layernorm(x_s[0].astype(F32)),
                                  _layernorm(tail(1))], axis=0)
    h_pre[0:L + PRE_ROWS, :] = first_rows.astype(BF16)
    for i in range(1, N_PRE, 2):
        two = jnp.concatenate([tail(i + 1), tail(i + 2)], axis=0)
        h_pre[L + i * PRE_ROWS:L + (i + 2) * PRE_ROWS, :] = _layernorm(two).astype(BF16)

    def land(g):
        for cp in stage_copies(g):
            cp.wait()

    def transposes(g, dst):
        slot = g % STAGE_DEPTH

        def piece(j, t):
            c0 = j * pw + t * 128
            dst[g // 2, :, c0:c0 + 128] = pltpu.bitcast(
                stage[slot, j, t * 128:(t + 1) * 128, :].T, U32)

        return [functools.partial(piece, j, t) for j in range(3) for t in range(n_tile)]

    def bulk(g, src, extra, first=0):
        n16 = h_pre.shape[0] // 16
        cuts = [16 * ((n16 * i) // 4) for i in range(5)]
        for i, pieces in enumerate(extra, first):
            for piece in pieces:
                piece()
            rows = slice(cuts[i], cuts[i + 1])
            pre[g, rows, :] = _mm(h_pre[rows, :], _w(src[g // 2]))

    land(0)
    for piece in transposes(0, wqkv_even):
        piece()
    bulk(0, wqkv_even, [[], []])
    land(1)
    for g in range(2, STAGE_DEPTH + 1):
        for cp in stage_copies(g):
            cp.start()

    def load_two(i, carry):
        for k, (src, dst) in enumerate(((wqkv_even, wqkv_odd), (wqkv_odd, wqkv_even))):
            g = 2 * i + 1 + k
            bulk(g - 1, src, [transposes(g, dst), []], 2)
            bulk(g, dst, [[], []])

            @pl.when(g + STAGE_DEPTH < n_pair)
            def _():
                for cp in stage_copies(g + STAGE_DEPTH):
                    cp.start()

            queued = lambda t: jnp.minimum((5 * t) // 4, n_pair)
            for j in range(2):
                @pl.when(queued(g - 1) + j < queued(g))
                def _():
                    wo_copy(queued(g - 1) + j).start()

            land(g + 1)
        return carry

    lax.fori_loop(0, n_pair // 2 - 1, load_two, 0)
    for cp in ffn_cps + [x_rest]:
        cp.start()
    pltpu.make_async_copy(wo_raw, wo_raw, sem_wo).wait()

    split, probs = make_attention()
    held, p, outs = {}, {}, {}

    def attend(i):
        if i < n_pair:
            held[i] = split(pre[i, 0:L, :])
            p[i] = probs(held[i][0], held[i][1])
        if i >= 4:
            outs[i - 4] = _mm(p.pop(i - 4), held.pop(i - 4)[2])

    att = [functools.partial(attend, i) for i in range(n_pair + 4)]
    bulk(n_pair - 2, wqkv_even, [transposes(n_pair - 1, wqkv_odd) + att[0:4], att[4:8]], 2)
    bulk(n_pair - 1, wqkv_odd, [att[8:12], att[12:16]])
    acc = None
    for g in range(n_pair):
        if g < 4:
            att[n_pair + g]()
        w = wo_raw[g]
        wo_s[g] = pltpu.bitcast(w, U32)
        t = _mm(outs.pop(g), w)
        acc = t if acc is None else acc + t
    finish(0, acc, 0, 0, 1)
    bulk(n_pair - 1, wqkv_odd, [[]], 2)

    step(1, 0, 1, 2, False, True)
    bulk(n_pair - 1, wqkv_odd, [[]], 3)
    for cp in ffn_cps + [x_rest]:
        cp.wait()

    def block(b, slot, short):
        hres[1 - slot] = step(2 * b, slot, 0, 2 * b + 1, True, short)
        res = step(2 * b + 1, slot, 1, jnp.minimum(2 * b + 2, n_seg - 1), True, short)
        out_s[pl.ds(pl.multiple_of((b - 1) * blk, blk), blk), :] = res.astype(BF16)

    def run(b0, b1, unroll, short):
        def body(i, carry):
            b = b0 + i * unroll
            for j in range(unroll):
                block(b + j, (b0 + j) % 2 if unroll % 2 == 0 else (b + j) % 2, short)
            for j in range(unroll):
                out_copy(b + j - 1).start()
            return carry
        lax.fori_loop(0, (b1 - b0) // unroll, body, 0)

    n_short = (N_PRE + 1) // 2
    run(1, n_short, UNROLL[0], True)
    run(n_short, n_blk, UNROLL[1], False)

    last = n_blk - 1
    a = hn[last % 2]
    acts = [_swiglu(_mm(a, wg_s[c]), _mm(a, wu_s[c])) for c in range(2)]
    res = hres[last % 2] + _mm(acts[0], wd_s[0]) + _mm(acts[1], wd_s[1])
    out_s[last * blk:(last + 1) * blk, :] = res.astype(BF16)
    out_copy(last).start()
    pltpu.make_async_copy(out_s, out_s, sem_out).wait()


@functools.partial(jax.jit, static_argnames=("A_seg_len",))
def pallas_sequential_preLN__memory_aug_recurrent_mem_tr__swiglu_ffn__prompt_kernel(
    A_x: jax.Array,
    A_mem0: jax.Array,
    A_Wq: jax.Array,
    A_Wk: jax.Array,
    A_Wv: jax.Array,
    A_Wo: jax.Array,
    A_seg_len: int,
    B_x: jax.Array,
    B_w_gate: jax.Array,
    B_w_up: jax.Array,
    B_w_down: jax.Array,
):
    del B_x
    batch, seq, d = A_x.shape
    _, heads, dh = A_Wq.shape
    n_mem = A_mem0.shape[1]
    seg = int(A_seg_len)
    n_seg = seq // seg
    f = B_w_gate.shape[1]
    n_pair = heads // 2
    pw = 2 * dh
    f_half = f // 2
    assert batch == 1 and n_seg * seg == seq and n_seg % 2 == 0 and n_seg > N_PRE + 3
    assert dh == 192 and heads == 32 and 2 * (n_mem + seg) <= 128 and f_half % FFN_COLS == 0

    wt = lambda w: jnp.transpose(w, (1, 2, 0)).reshape(heads * dh, d)

    hbm = pl.BlockSpec(memory_space=pl.ANY)
    n_rows = n_mem + seg + N_PRE * PRE_ROWS
    body = functools.partial(_kernel, n_seg=n_seg, seg=seg, n_mem=n_mem, n_pair=n_pair,
                             dh=dh, f_half=f_half)
    out = pl.pallas_call(
        body,
        out_shape=jax.ShapeDtypeStruct((seq, d), A_x.dtype),
        in_specs=[hbm] * 9,
        out_specs=hbm,
        scratch_shapes=[
            pltpu.VMEM((STAGE_DEPTH, 3, pw, d), BF16),
            pltpu.VMEM((n_pair // 2, d // 2, 3 * pw), U32),
            pltpu.VMEM((n_pair // 2, d // 2, 3 * pw), U32),
            pltpu.VMEM((n_pair, pw, d), BF16),
            pltpu.VMEM((n_pair, pw // 2, d), U32),
            pltpu.VMEM((2, d, f_half), BF16),
            pltpu.VMEM((2, d, f_half), BF16),
            pltpu.VMEM((2, f_half, d), BF16),
            pltpu.VMEM((n_seg, seg, d), BF16),
            pltpu.VMEM((N_PRE, PRE_ROWS, d), BF16),
            pltpu.VMEM((n_mem, d), BF16),
            pltpu.VMEM((n_rows, d), BF16),
            pltpu.VMEM((n_pair, n_rows, 3 * pw), F32),
            pltpu.VMEM((n_mem + seg, d), F32),
            pltpu.VMEM((2, 2 * seg, d), F32),
            pltpu.VMEM((2, 2 * seg, d), BF16),
            pltpu.VMEM((seq, d), BF16),
            pltpu.SemaphoreType.DMA((STAGE_DEPTH * 3,)),
            pltpu.SemaphoreType.DMA(()),
            pltpu.SemaphoreType.DMA((10,)),
            pltpu.SemaphoreType.DMA(()),
        ],
        compiler_params=pltpu.CompilerParams(vmem_limit_bytes=120 * 1024 * 1024, flags={'XLA_TPU_EVENLY_DISTRIBUTE_CRITICAL_NODES': True}),
    )(A_x.reshape(n_seg, seg, d), A_mem0.reshape(n_mem, d), wt(A_Wq), wt(A_Wk), wt(A_Wv),
      A_Wo.reshape(heads * dh, d), B_w_gate, B_w_up, B_w_down)
    return out.reshape(batch, seq, d)
```

```python
import functools

import jax
import jax.numpy as jnp
from jax import lax
import jax.experimental.pallas as pl
import jax.experimental.pallas.tpu as pltpu

F32 = jnp.float32
BF16 = jnp.bfloat16
U32 = jnp.uint32

LN_EPS = 1e-5
MASK_VALUE = -1000000000.0
STAGE_DEPTH = 4
PRE_ROWS = 8
N_PRE = 43
FFN_COLS = 384
LAG_QK = 1
LAG_PV = 3


def _mm(a, b):
    return lax.dot_general(a, b, (((1,), (0,)), ((), ())), preferred_element_type=F32)


def _mm_t(a, b):
    return lax.dot_general(a, b, (((1,), (1,)), ((), ())), preferred_element_type=F32)


def _w(packed):
    return pltpu.bitcast(packed, BF16)


def _swiglu(gate, up):
    hg = 0.5 * gate
    return ((hg * jnp.tanh(hg) + hg) * up).astype(BF16)


def _recip(x):
    r = pl.reciprocal(x, approx=True)
    return r * (2.0 - x * r)


def _layernorm(x):
    n = x.shape[-1]
    mean = jnp.sum(x, axis=-1, keepdims=True) * (1.0 / n)
    d = x - mean
    var = jnp.sum(d * d, axis=-1, keepdims=True) * (1.0 / n)
    return d * lax.rsqrt(var + LN_EPS)


def _kernel(x_hbm, mem0_hbm, wq_hbm, wk_hbm, wv_hbm, wo_hbm, wg_hbm, wu_hbm, wd_hbm,
            out_hbm,
            stage, wqkv_even, wqkv_odd, wo_raw, wo_s, wg_s, wu_s, wd_s,
            x_s, x_pre, mem_s, h_pre, pre, hbuf, hres, hn, out_s,
            sem_stage, sem_wo, sem_misc, sem_out,
            *, n_seg, seg, n_mem, n_pair, dh, f_half):
    L = n_mem + seg
    pw = 2 * dh
    n_tile = pw // 128
    blk = 2 * seg
    n_blk = n_seg // 2
    scale = dh ** (-0.5)
    live = seg - PRE_ROWS

    def pair_rows(g):
        return pl.ds(pl.multiple_of(g * pw, 128), pw)

    def stage_copies(g):
        slot = g % STAGE_DEPTH
        return [pltpu.make_async_copy(w.at[pair_rows(g), :], stage.at[slot, j],
                                      sem_stage.at[slot * 3 + j])
                for j, w in enumerate((wq_hbm, wk_hbm, wv_hbm))]

    def wo_copy(g):
        return pltpu.make_async_copy(wo_hbm.at[pair_rows(g), :], wo_raw.at[g], sem_wo)

    def out_copy(b):
        rows = pl.ds(pl.multiple_of(b * blk, blk), blk)
        return pltpu.make_async_copy(out_s.at[rows, :], out_hbm.at[rows, :], sem_out)

    mem_cp = pltpu.make_async_copy(mem0_hbm, mem_s, sem_misc.at[8])
    x_head = pltpu.make_async_copy(x_hbm.at[pl.ds(0, 3)], x_s.at[pl.ds(0, 3)], sem_misc.at[0])
    x_rest = pltpu.make_async_copy(x_hbm.at[pl.ds(3, n_seg - 3)], x_s.at[pl.ds(3, n_seg - 3)],
                                   sem_misc.at[1])
    x_tail = pltpu.make_async_copy(x_hbm.at[pl.ds(1, N_PRE), pl.ds(live, PRE_ROWS), :], x_pre,
                                   sem_misc.at[9])
    ffn_cps = []
    for c in range(2):
        cols = pl.ds(c * f_half, f_half)
        ffn_cps.append(pltpu.make_async_copy(wg_hbm.at[:, cols], wg_s.at[c], sem_misc.at[2 + c]))
        ffn_cps.append(pltpu.make_async_copy(wu_hbm.at[:, cols], wu_s.at[c], sem_misc.at[4 + c]))
        ffn_cps.append(pltpu.make_async_copy(wd_hbm.at[cols, :], wd_s.at[c], sem_misc.at[6 + c]))

    def w_qkv(g):
        return _w((wqkv_odd if g % 2 else wqkv_even)[g // 2])

    def make_attention():
        row = lax.broadcasted_iota(jnp.int32, (L, 128), 0)
        col = lax.broadcasted_iota(jnp.int32, (L, 128), 1)
        first = col < L
        second = (col >= L) & (col < 2 * L)
        key = jnp.where(first, col, col - L)
        visible = (row < n_mem) | (row >= key)
        lo = col < (dh - 128)
        zeros = jnp.zeros((L, 128), F32)

        def split(r):
            k0, k1, k2, v0, v1, v2 = (r[:, t * 128:(t + 1) * 128]
                                      for t in range(n_tile, 3 * n_tile))
            k01 = jnp.concatenate([
                jnp.concatenate([k0, jnp.where(lo, k1, 0.0)], axis=1),
                jnp.concatenate([zeros, jnp.where(lo, 0.0, k1)], axis=1),
                jnp.zeros((128 - 2 * L, 256), F32)], axis=0).astype(BF16)
            k2 = jnp.concatenate([k2, jnp.zeros((128 - L, 128), F32)], axis=0).astype(BF16)
            vb = jnp.concatenate([
                jnp.concatenate([v0, jnp.where(lo, v1, 0.0), zeros], axis=1),
                jnp.concatenate([zeros, jnp.where(lo, 0.0, v1), v2], axis=1)], axis=0).astype(BF16)
            return r[:, 0:pw], (k01, k2), vb

        def probs(q, k):
            sc = _mm_t(q[:, 0:256], k[0]) + pltpu.roll(_mm_t(q[:, 256:384], k[1]), L, axis=1)
            sc = jnp.where(visible, sc * scale, MASK_VALUE)
            m_a = jnp.max(jnp.where(first, sc, -jnp.inf), axis=1, keepdims=True)
            m_b = jnp.max(jnp.where(second, sc, -jnp.inf), axis=1, keepdims=True)
            e = jnp.exp(sc - jnp.where(first, m_a, m_b))
            l_a = jnp.sum(jnp.where(first, e, 0.0), axis=1, keepdims=True)
            l_b = jnp.sum(jnp.where(second, e, 0.0), axis=1, keepdims=True)
            return (e * _recip(jnp.where(first, l_a, l_b)))[:, 0:2 * L]

        return split, probs

    def finish(s, acc, slot, c, nxt):
        hbuf[0:n_mem, :] = acc[0:n_mem, :]
        hbuf[n_mem:L, :] = _layernorm(x_s[nxt].astype(F32))
        h = x_s[s].astype(F32) + acc[n_mem:L, :]
        hres[slot, c * seg:(c + 1) * seg, :] = h
        hn[slot, c * seg:(c + 1) * seg, :] = _layernorm(h).astype(BF16)

    def step(s, slot, c, nxt, with_ffn, short):
        split, probs = make_attention()
        if short:
            h = hbuf[0:n_mem + live, :].astype(BF16)
            ready = pl.ds(pl.multiple_of(L + (s - 1) * PRE_ROWS, PRE_ROWS), PRE_ROWS)
            project = lambda g: jnp.concatenate([_mm(h, w_qkv(g)), pre[g, ready, :]], axis=0)
        else:
            h = hbuf[...]
            project = lambda g: _mm(h, w_qkv(g))
        held, p, outs = {}, {}, {}

        def attend(i):
            if 0 <= i - LAG_PV < n_pair:
                outs[i - LAG_PV] = _mm(p.pop(i - LAG_PV), held.pop(i - LAG_PV)[2])
            if 0 <= i - LAG_QK < n_pair:
                p[i - LAG_QK] = probs(held[i - LAG_QK][0], held[i - LAG_QK][1])

        for i in range(n_pair):
            held[i] = split(project(i))
            attend(i)
        acc = None
        acts = []
        if with_ffn:
            a = hn[1 - slot]
        for g in range(n_pair):
            if with_ffn and g % 3 == 0 and g // 3 < f_half // FFN_COLS:
                cs = slice((g // 3) * FFN_COLS, (g // 3 + 1) * FFN_COLS)
                acts.append(_swiglu(_mm(a, wg_s[c, :, cs]), _mm(a, wu_s[c, :, cs])))
            if g % 3 == (0 if with_ffn else 2):
                attend(n_pair + g // 3)
            t = _mm(outs.pop(g), _w(wo_s[g]))
            acc = t if acc is None else acc + t
        finish(s, acc, slot, c, nxt)
        if with_ffn:
            return hres[1 - slot] + _mm(jnp.concatenate(acts, axis=1), wd_s[c])

    for cp in [mem_cp, x_head, x_tail] + stage_copies(0):
        cp.start()
    mem_cp.wait()
    x_head.wait()
    for cp in stage_copies(1):
        cp.start()
    x_tail.wait()
    tail = lambda i: x_pre[i - 1].astype(F32)
    first_rows = jnp.concatenate([mem_s[...].astype(F32), _layernorm(x_s[0].astype(F32)),
                                  _layernorm(tail(1))], axis=0)
    h_pre[0:L + PRE_ROWS, :] = first_rows.astype(BF16)
    for i in range(1, N_PRE, 2):
        two = jnp.concatenate([tail(i + 1), tail(i + 2)], axis=0)
        h_pre[L + i * PRE_ROWS:L + (i + 2) * PRE_ROWS, :] = _layernorm(two).astype(BF16)

    def land(g):
        for cp in stage_copies(g):
            cp.wait()

    def transposes(g, dst):
        slot = g % STAGE_DEPTH

        def piece(j, t):
            c0 = j * pw + t * 128
            dst[g // 2, :, c0:c0 + 128] = pltpu.bitcast(
                stage[slot, j, t * 128:(t + 1) * 128, :].T, U32)

        return [functools.partial(piece, j, t) for j in range(3) for t in range(n_tile)]

    def bulk(g, src, extra, first=0):
        n16 = h_pre.shape[0] // 16
        cuts = [16 * ((n16 * i) // 4) for i in range(5)]
        for i, pieces in enumerate(extra, first):
            for piece in pieces:
                piece()
            rows = slice(cuts[i], cuts[i + 1])
            pre[g, rows, :] = _mm(h_pre[rows, :], _w(src[g // 2]))

    land(0)
    for piece in transposes(0, wqkv_even):
        piece()
    bulk(0, wqkv_even, [[], []])
    land(1)
    for g in range(2, STAGE_DEPTH + 1):
        for cp in stage_copies(g):
            cp.start()

    def load_two(i, carry):
        for k, (src, dst) in enumerate(((wqkv_even, wqkv_odd), (wqkv_odd, wqkv_even))):
            g = 2 * i + 1 + k
            bulk(g - 1, src, [transposes(g, dst), []], 2)
            bulk(g, dst, [[], []])

            @pl.when(g + STAGE_DEPTH < n_pair)
            def _():
                for cp in stage_copies(g + STAGE_DEPTH):
                    cp.start()

            queued = lambda t: jnp.minimum((5 * t) // 4, n_pair)
            for j in range(2):
                @pl.when(queued(g - 1) + j < queued(g))
                def _():
                    wo_copy(queued(g - 1) + j).start()

            land(g + 1)
        return carry

    lax.fori_loop(0, n_pair // 2 - 1, load_two, 0)
    for cp in ffn_cps + [x_rest]:
        cp.start()
    for g in range(n_pair):
        wo_copy(g).wait()

    split, probs = make_attention()
    held, p, outs = {}, {}, {}

    def attend0(i):
        if i < n_pair:
            held[i] = split(pre[i, 0:L, :])
            p[i] = probs(held[i][0], held[i][1])
        if i >= 4:
            outs[i - 4] = _mm(p.pop(i - 4), held.pop(i - 4)[2])

    att = [functools.partial(attend0, i) for i in range(n_pair + 4)]
    bulk(n_pair - 2, wqkv_even, [transposes(n_pair - 1, wqkv_odd) + att[0:4], att[4:8]], 2)
    bulk(n_pair - 1, wqkv_odd, [att[8:12], att[12:16]])
    acc = None
    for g in range(n_pair):
        if g < 4:
            att[n_pair + g]()
        w = wo_raw[g]
        wo_s[g] = pltpu.bitcast(w, U32)
        t = _mm(outs.pop(g), w)
        acc = t if acc is None else acc + t
    finish(0, acc, 0, 0, 1)
    bulk(n_pair - 1, wqkv_odd, [[]], 2)

    step(1, 0, 1, 2, False, True)
    bulk(n_pair - 1, wqkv_odd, [[]], 3)
    for cp in ffn_cps + [x_rest]:
        cp.wait()

    def block(b, carry, short):
        slot = b % 2
        hres[1 - slot] = step(2 * b, slot, 0, 2 * b + 1, True, short)
        res = step(2 * b + 1, slot, 1, jnp.minimum(2 * b + 2, n_seg - 1), True, short)
        out_s[pl.ds(pl.multiple_of((b - 1) * blk, blk), blk), :] = res.astype(BF16)
        out_copy(b - 1).start()
        return carry

    n_short = (N_PRE + 1) // 2
    lax.fori_loop(1, n_short, functools.partial(block, short=True), 0)
    lax.fori_loop(n_short, n_blk, functools.partial(block, short=False), 0)

    last = n_blk - 1
    a = hn[last % 2]
    acts = [_swiglu(_mm(a, wg_s[c]), _mm(a, wu_s[c])) for c in range(2)]
    res = hres[last % 2] + _mm(acts[0], wd_s[0]) + _mm(acts[1], wd_s[1])
    out_s[last * blk:(last + 1) * blk, :] = res.astype(BF16)
    out_copy(last).start()
    for b in range(n_blk):
        out_copy(b).wait()


@functools.partial(jax.jit, static_argnames=("A_seg_len",))
def pallas_sequential_preLN__memory_aug_recurrent_mem_tr__swiglu_ffn__prompt_kernel(
    A_x: jax.Array,
    A_mem0: jax.Array,
    A_Wq: jax.Array,
    A_Wk: jax.Array,
    A_Wv: jax.Array,
    A_Wo: jax.Array,
    A_seg_len: int,
    B_x: jax.Array,
    B_w_gate: jax.Array,
    B_w_up: jax.Array,
    B_w_down: jax.Array,
):
    del B_x
    batch, seq, d = A_x.shape
    _, heads, dh = A_Wq.shape
    n_mem = A_mem0.shape[1]
    seg = int(A_seg_len)
    n_seg = seq // seg
    f = B_w_gate.shape[1]
    n_pair = heads // 2
    pw = 2 * dh
    f_half = f // 2
    assert batch == 1 and n_seg * seg == seq and n_seg % 2 == 0 and n_seg > N_PRE + 3
    assert dh == 192 and heads == 32 and 2 * (n_mem + seg) <= 128 and f_half % FFN_COLS == 0

    wt = lambda w: jnp.transpose(w, (1, 2, 0)).reshape(heads * dh, d)

    hbm = pl.BlockSpec(memory_space=pl.ANY)
    n_rows = n_mem + seg + N_PRE * PRE_ROWS
    body = functools.partial(_kernel, n_seg=n_seg, seg=seg, n_mem=n_mem, n_pair=n_pair,
                             dh=dh, f_half=f_half)
    out = pl.pallas_call(
        body,
        out_shape=jax.ShapeDtypeStruct((seq, d), A_x.dtype),
        in_specs=[hbm] * 9,
        out_specs=hbm,
        scratch_shapes=[
            pltpu.VMEM((STAGE_DEPTH, 3, pw, d), BF16),
            pltpu.VMEM((n_pair // 2, d // 2, 3 * pw), U32),
            pltpu.VMEM((n_pair // 2, d // 2, 3 * pw), U32),
            pltpu.VMEM((n_pair, pw, d), BF16),
            pltpu.VMEM((n_pair, pw // 2, d), U32),
            pltpu.VMEM((2, d, f_half), BF16),
            pltpu.VMEM((2, d, f_half), BF16),
            pltpu.VMEM((2, f_half, d), BF16),
            pltpu.VMEM((n_seg, seg, d), BF16),
            pltpu.VMEM((N_PRE, PRE_ROWS, d), BF16),
            pltpu.VMEM((n_mem, d), BF16),
            pltpu.VMEM((n_rows, d), BF16),
            pltpu.VMEM((n_pair, n_rows, 3 * pw), F32),
            pltpu.VMEM((n_mem + seg, d), F32),
            pltpu.VMEM((2, 2 * seg, d), F32),
            pltpu.VMEM((2, 2 * seg, d), BF16),
            pltpu.VMEM((seq, d), BF16),
            pltpu.SemaphoreType.DMA((STAGE_DEPTH * 3,)),
            pltpu.SemaphoreType.DMA(()),
            pltpu.SemaphoreType.DMA((10,)),
            pltpu.SemaphoreType.DMA(()),
        ],
        compiler_params=pltpu.CompilerParams(vmem_limit_bytes=120 * 1024 * 1024),
    )(A_x.reshape(n_seg, seg, d), A_mem0.reshape(n_mem, d), wt(A_Wq), wt(A_Wk), wt(A_Wv),
      A_Wo.reshape(heads * dh, d), B_w_gate, B_w_up, B_w_down)
    return out.reshape(batch, seq, d)
```
